```python
import os as _os
_os.environ.setdefault("JAX_PLATFORMS", "cpu")
import jax
import jax.numpy as jnp

def _softmax(x, axis=-1):
    return jax.nn.softmax(x, axis=axis)
def _gelu(x):
    return jax.nn.gelu(x, approximate=True)
def _silu(x):
    return jax.nn.silu(x)
def _sigmoid(x):
    return jax.nn.sigmoid(x)
def _layernorm(x, axis=-1, eps=1e-5):
    m = jnp.mean(x, axis=axis, keepdims=True)
    v = jnp.var(x, axis=axis, keepdims=True)
    return (x - m) / jnp.sqrt(v + eps)
def _scatter_add(tgt, idx, src, axis=0):
    return tgt.at[idx].add(src)
def _segment_sum(src, seg, n):
    return jax.ops.segment_sum(src, seg, n)
class _Rng:
    def __init__(self, key):
        self._k = key
    def _next(self):
        self._k, sub = jax.random.split(self._k)
        return sub
    def normal(self, shape):
        return jax.random.normal(self._next(), shape, dtype=jnp.bfloat16)
    def randint(self, lo, hi, shape):
        return jax.random.randint(self._next(), shape, lo, hi, dtype=jnp.int32)
    def uniform(self, shape, lo=0.0, hi=1.0):
        return jax.random.uniform(self._next(), shape, jnp.bfloat16, lo, hi)
    def permutation(self, n):
        return jax.random.permutation(self._next(), n)


kernel_name = 'sequential_preLN__compressed_kv_cla__dense_activation_mish__decode'

def setup_inputs():
    _rng = _Rng(jax.random.key(int.from_bytes(__import__("os").urandom(4), "little")))
    _w = (lambda a: (lambda t: t.astype(jnp.bfloat16) if jnp.issubdtype(t.dtype, jnp.floating) else t)(jnp.asarray(a)))
    def _A_setup():
        B, H, Sq, Sk, D, M = 1, 32, 1, 8192, 128, 512
        Dc = 4 * D
        return {
            "x": _w((lambda *s: _rng.normal(s) * 0.05)(B, Sq, M)),
            "c_kv": _w((lambda *s: _rng.normal(s) * 0.8)(B, Sk, Dc)),
            "w_q": _w((lambda *s: _rng.normal(s) * 0.8)(M, H, D) * (M ** -0.5)),
            "w_uk": _w((lambda *s: _rng.normal(s) * 0.8)(Dc, H, D) * (Dc ** -0.5)),
            "w_uv": _w((lambda *s: _rng.normal(s) * 0.8)(Dc, H, D) * (Dc ** -0.5)),
            "w_o": _w((lambda *s: _rng.normal(s) * 0.8)(H, D, M) * ((H * D) ** -0.5)),
        }
    _A_in = _A_setup()

    def _B_setup():
        B, S, D, F = 1, 1, 512, 1376
        return {
            "x": _w((lambda *s: _rng.normal(s) * 0.05)(B, S, D)),
            "w1": _w((lambda *s: _rng.normal(s) * 0.2)(D, F) * (D ** -0.5)),
            "b1": _w((lambda *s: _rng.normal(s) * 0.05)(F)),
            "w2": _w((lambda *s: _rng.normal(s) * 0.05)(F, D) * (F ** -0.5)),
        }
    _B_in = _B_setup()

    return {
        "A_x": _A_in["x"],
        "A_c_kv": _A_in["c_kv"],
        "A_w_q": _A_in["w_q"],
        "A_w_uk": _A_in["w_uk"],
        "A_w_uv": _A_in["w_uv"],
        "A_w_o": _A_in["w_o"],
        "B_x": _B_in["x"],
        "B_w1": _B_in["w1"],
        "B_b1": _B_in["b1"],
        "B_w2": _B_in["w2"],
    }

def reference(A_x, A_c_kv, A_w_q, A_w_uk, A_w_uv, A_w_o, B_x, B_w1, B_b1, B_w2):
    def _A_ref(x, c_kv, w_q, w_uk, w_uv, w_o):
        B, Sq, M = x.shape[0], x.shape[1], x.shape[2]
        Sk = c_kv.shape[1]
        H, D = w_q.shape[1], w_q.shape[2]
        q = jnp.einsum("bqm,mhd->bhqd", x, w_q)
        k = jnp.einsum("bkc,chd->bhkd", c_kv, w_uk)
        v = jnp.einsum("bkc,chd->bhkd", c_kv, w_uv)
        scores = jnp.einsum("bhqd,bhkd->bhqk", q, k) * (D ** -0.5)
        off = Sk - Sq
        qi = jnp.arange(Sq)[:, None]
        kj = jnp.arange(Sk)[None, :]
        cmask = kj <= (qi + off)
        scores = jnp.where(cmask[None, None], scores, -1e9)
        p = _softmax(scores, axis=-1)
        ctx = jnp.einsum("bhqk,bhkd->bhqd", p, v)
        return jnp.einsum("bhqd,hdm->bqm", ctx, w_o)

    def _B_ref(x, w1, b1, w2):
        h = jnp.einsum("bsd,df->bsf", x, w1) + b1
        sp = jnp.log1p(jnp.exp(-jnp.abs(h))) + jnp.where(h > 0, h, jnp.zeros_like(h))
        act = h * jnp.tanh(sp)
        return jnp.einsum("bsf,fd->bsd", act, w2)

    x = A_x
    h = x + _A_ref(_layernorm(x, axis=-1), A_c_kv, A_w_q, A_w_uk, A_w_uv, A_w_o)
    h2 = h + _B_ref(_layernorm(h, axis=-1), B_w1, B_b1, B_w2)
    return h2
```

```python
import functools
import jax
import jax.numpy as jnp
import numpy as np
from jax import lax
from jax.experimental import pallas as pl
from jax.experimental.pallas import tpu as pltpu

F32 = jnp.float32
BF16 = jnp.bfloat16
M = 512; H = 32; D = 128; SK = 8192; DC = 512; FF = 1376
NKV = 8
KVC = SK // NKV
W2_SPLITS = (0, 640, 1152, 1376)

def _nt(a, b):
    return lax.dot_general(a, b, (((1,), (1,)), ((), ())), preferred_element_type=F32)
def _nn(a, b):
    return jnp.dot(a, b, preferred_element_type=F32)

def _ln(x):
    m = jnp.mean(x, axis=-1, keepdims=True)
    xc = x - m
    v = jnp.mean(xc * xc, axis=-1, keepdims=True)
    return xc / jnp.sqrt(v + 1e-5)

def kernel(x_h, ckv_h, wq_h, wuk_h, wuv_h, wo_h, w1t_h, b1_h, w2_h, o_ref,
           x_v, b1_v, ckv_v, wq_v, wuk_v, wuv_v, wo_v, w1_v, w2_v, cp_v, s_v, p_v, ctx_v, sems):
    cps = []
    def mk(src, dst):
        c = pltpu.make_async_copy(src, dst, sems.at[len(cps)])
        cps.append(c)
        return c
    c_x = mk(x_h, x_v)
    c_b1 = mk(b1_h, b1_v)
    c_wq = [mk(wq_h.at[pl.ds(i * 4096, 4096)], wq_v.at[pl.ds(i * 4096, 4096)]) for i in range(4)]
    c_wuk = [mk(wuk_h.at[pl.ds(i * 4096, 4096)], wuk_v.at[pl.ds(i * 4096, 4096)]) for i in range(4)]
    c_kv = [mk(ckv_h.at[pl.ds(i * KVC, KVC)], ckv_v.at[pl.ds(i * KVC, KVC)]) for i in range(NKV)]
    c_wuv = [mk(wuv_h.at[pl.ds(i * 4096, 4096)], wuv_v.at[pl.ds(i * 4096, 4096)]) for i in range(4)]
    c_wo = [mk(wo_h.at[pl.ds(i * 1024, 1024)], wo_v.at[pl.ds(i * 1024, 1024)]) for i in range(4)]
    c_w1 = mk(w1t_h, w1_v)
    c_w2 = [mk(w2_h.at[pl.ds(a, b - a)], w2_v.at[pl.ds(a, b - a)]) for a, b in zip(W2_SPLITS[:-1], W2_SPLITS[1:])]
    for c in cps:
        c.start()

    row = lax.broadcasted_iota(jnp.int32, (H, 128), 0)
    lane = lax.broadcasted_iota(jnp.int32, (H, 128), 1)
    diag = (lane % H) == row
    pr = lax.broadcasted_iota(jnp.int32, (128, 128), 0)
    pc = lax.broadcasted_iota(jnp.int32, (128, 128), 1)
    perm = (pc == (pr % 4) * 32 + pr // 4).astype(F32).astype(BF16)

    def permute_cols(a_bf16):
        return [_nn(a_bf16[:, T * 128:(T + 1) * 128], perm) for T in range(4)]

    def expand_matmul(cp, w_ref):
        tiles = []
        g = pltpu.roll(cp, 0, 1, stride=1, stride_axis=0)
        for t in range(32):
            r = pltpu.roll(g, (128 - t) % 128, 1) if t else g
            tiles.append(jnp.where(diag, r, 0.0).astype(BF16))
        s = jnp.concatenate(tiles, axis=1)
        return _nn(s, w_ref)

    c_x.wait()
    x = x_v[0].astype(F32)
    xn = _ln(x).astype(BF16)
    xb = jnp.broadcast_to(xn, (H, M))
    cps0 = permute_cols(xb)
    q = jnp.zeros((H, D), F32)
    for T in range(4):
        c_wq[T].wait()
        q = q + expand_matmul(cps0[T], wq_v[pl.ds(T * 4096, 4096), :])
    qb = q.astype(BF16)
    qa_parts = []
    for T in range(4):
        c_wuk[T].wait()
        z = _nt(qb, wuk_v[pl.ds(T * 4096, 4096), :])
        acc = jnp.zeros((H, 128), F32)
        for t in range(32):
            zt = jnp.where(diag, z[:, t * 128:(t + 1) * 128], 0.0)
            acc = acc + (pltpu.roll(zt, t, 1) if t else zt)
        for b in range(5):
            acc = jnp.where((row >> b) & 1 == 1, pltpu.roll(acc, 128 - (1 << b), 1), acc)
        qa_parts.append(_nt(acc.astype(BF16), perm))
    qa = (jnp.concatenate(qa_parts, axis=1) * (D ** -0.5)).astype(BF16)
    mx = jnp.full((H, 128), -jnp.inf, F32)
    for i in range(NKV):
        c_kv[i].wait()
        s = _nt(qa, ckv_v[pl.ds(i * KVC, KVC), :])
        s_v[:, pl.ds(i * KVC, KVC)] = s
        for j in range(KVC // 128):
            mx = jnp.maximum(mx, s[:, j * 128:(j + 1) * 128])
    mxr = jnp.max(mx, axis=-1, keepdims=True)
    lsum = jnp.zeros((H, 128), F32)
    cl = jnp.zeros((H, DC), F32)
    for i in range(NKV):
        p = jnp.exp(s_v[:, pl.ds(i * KVC, KVC)] - mxr)
        for j in range(KVC // 128):
            lsum = lsum + p[:, j * 128:(j + 1) * 128]
        cl = cl + _nn(p.astype(BF16), ckv_v[pl.ds(i * KVC, KVC), :])
    l = jnp.sum(lsum, axis=-1, keepdims=True)
    cl = (cl / l).astype(BF16)
    cps4 = permute_cols(cl)
    ctx = jnp.zeros((H, D), F32)
    for T in range(4):
        c_wuv[T].wait()
        ctx = ctx + expand_matmul(cps4[T], wuv_v[pl.ds(T * 4096, 4096), :])
    ctx_v[...] = ctx
    hacc = x
    for g in range(4):
        c_wo[g].wait()
        lhs = jnp.concatenate([ctx_v[pl.ds(g * 8 + k, 1), :] for k in range(8)], axis=1).astype(BF16)
        hacc = hacc + _nn(lhs, wo_v[pl.ds(g * 1024, 1024), :])
    hn = _ln(hacc).astype(BF16)
    c_w1.wait()
    c_b1.wait()
    hh = _nt(hn, w1_v[...]) + b1_v[...].astype(F32).reshape(1, FF)
    sp = jnp.log1p(jnp.exp(-jnp.abs(hh))) + jnp.maximum(hh, 0.0)
    act = (hh * jnp.tanh(sp)).astype(BF16)
    out = hacc
    for c, a, b in zip(c_w2, W2_SPLITS[:-1], W2_SPLITS[1:]):
        c.wait()
        out = out + _nn(act[:, a:b], w2_v[pl.ds(a, b - a), :])
    o_ref[0] = out.astype(BF16)

NDMA = 2 + 4 + 4 + NKV + 4 + 4 + 1 + len(W2_SPLITS) - 1

@jax.jit
def pallas_sequential_preLN__compressed_kv_cla__dense_activation_mish__decode_kernel(A_x, A_c_kv, A_w_q, A_w_uk, A_w_uv, A_w_o, B_x, B_w1, B_b1, B_w2):
    hbm = pl.BlockSpec(memory_space=pltpu.HBM)
    return pl.pallas_call(
        kernel,
        out_shape=jax.ShapeDtypeStruct((1, 1, M), BF16),
        in_specs=[hbm] * 9,
        out_specs=pl.BlockSpec(memory_space=pltpu.VMEM),
        scratch_shapes=[
            pltpu.VMEM((1, 1, M), BF16),
            pltpu.VMEM((FF,), BF16),
            pltpu.VMEM((SK, DC), BF16),
            pltpu.VMEM((M * H, D), BF16),
            pltpu.VMEM((DC * H, D), BF16),
            pltpu.VMEM((DC * H, D), BF16),
            pltpu.VMEM((H * D, M), BF16),
            pltpu.VMEM((FF, M), BF16),
            pltpu.VMEM((FF, M), BF16),
            pltpu.VMEM((H, DC), F32),
            pltpu.VMEM((H, SK), F32),
            pltpu.VMEM((H, SK), BF16),
            pltpu.VMEM((H, D), F32),
            pltpu.SemaphoreType.DMA((NDMA,)),
        ],
        compiler_params=pltpu.CompilerParams(vmem_limit_bytes=100 * 1024 * 1024),
    )(A_x, A_c_kv.reshape(SK, DC), A_w_q.reshape(M * H, D), A_w_uk.reshape(DC * H, D),
      A_w_uv.reshape(DC * H, D), A_w_o.reshape(H * D, M), B_w1.T, B_b1, B_w2)
```

```python
import functools

import jax
import jax.numpy as jnp
from jax import lax
from jax.experimental import pallas as pl
from jax.experimental.pallas import tpu as pltpu

F32 = jnp.float32
BF16 = jnp.bfloat16

M = 512
H = 32
D = 128
SK = 8192
DC = 512
FF = 1376
LANES = 128
CPT = LANES // H
NT = LANES // CPT
KV_STEP = 1024
W2_SPLITS = (0, 1024, 1280, FF)
N_DMA = 8 + len(W2_SPLITS) - 1
EPS = 1e-5


def _nn(a, b):
    return jnp.dot(a, b, preferred_element_type=F32)


def _nt(a, b):
    return lax.dot_general(a, b, (((1,), (1,)), ((), ())), preferred_element_type=F32)


def _layernorm(x):
    mean = jnp.mean(x, axis=-1, keepdims=True)
    xc = x - mean
    var = jnp.mean(xc * xc, axis=-1, keepdims=True)
    return xc / jnp.sqrt(var + EPS)


def _body(x_h, ckv_h, wq_h, wuk_h, wuv_h, wo_h, w1t_h, b1_h, w2_h, o_ref,
          x_v, b1_v, ckv_v, wq_v, wuk_v, wuv_v, wo_v, w1_v, w2_v, s_v, ctx_v, sems):
    copies = []

    def copy(src, dst):
        c = pltpu.make_async_copy(src, dst, sems.at[len(copies)])
        copies.append(c)
        return c

    c_wq = copy(wq_h, wq_v)
    c_x = copy(x_h, x_v)
    c_b1 = copy(b1_h, b1_v)
    c_wuk = copy(wuk_h, wuk_v)
    c_kv = copy(ckv_h, ckv_v)
    c_wuv = copy(wuv_h, wuv_v)
    c_wo = copy(wo_h, wo_v)
    c_w1 = copy(w1t_h, w1_v)
    w2_parts = list(zip(W2_SPLITS[:-1], W2_SPLITS[1:]))
    c_w2 = [copy(w2_h.at[pl.ds(a, b - a)], w2_v.at[pl.ds(a, b - a)]) for a, b in w2_parts]
    for c in copies:
        c.start()

    row = lax.broadcasted_iota(jnp.int32, (H, LANES), 0)
    lane = lax.broadcasted_iota(jnp.int32, (H, LANES), 1)
    diag = (lane % H) == row
    pr = lax.broadcasted_iota(jnp.int32, (LANES, LANES), 0)
    pc = lax.broadcasted_iota(jnp.int32, (LANES, LANES), 1)
    perm = (pc == (pr % CPT) * H + pr // CPT).astype(F32).astype(BF16)
    blk = LANES * H

    def head_matvec(s_bf16, w_ref):
        out = jnp.zeros((H, D), F32)
        for b in range(DC // LANES):
            sp = _nn(s_bf16[:, b * LANES:(b + 1) * LANES], perm)
            g = pltpu.roll(sp, 0, 1, stride=1, stride_axis=0)
            tiles = []
            for t in range(NT):
                r = pltpu.roll(g, LANES - t, 1) if t else g
                tiles.append(jnp.where(diag, r, 0.0).astype(BF16))
            out = out + _nn(jnp.concatenate(tiles, axis=1), w_ref[pl.ds(b * blk, blk), :])
        return out

    c_x.wait()
    x = x_v[0].astype(F32)
    xn = _layernorm(x).astype(BF16)
    xn_b = jnp.broadcast_to(xn, (H, M))
    c_wq.wait()
    q = head_matvec(xn_b, wq_v)
    qb = (q * (D ** -0.5)).astype(BF16)

    c_wuk.wait()
    qa_parts = []
    for b in range(DC // LANES):
        z = _nt(qb, wuk_v[pl.ds(b * blk, blk), :])
        acc = jnp.zeros((H, LANES), F32)
        for t in range(NT):
            zt = jnp.where(diag, z[:, t * LANES:(t + 1) * LANES], 0.0)
            acc = acc + (pltpu.roll(zt, t, 1) if t else zt)
        for bit in range(5):
            take = ((row >> bit) & 1) == 1
            acc = jnp.where(take, pltpu.roll(acc, LANES - (1 << bit), 1), acc)
        qa_parts.append(_nt(acc.astype(BF16), perm))
    qa = jnp.concatenate(qa_parts, axis=1).astype(BF16)

    c_kv.wait()
    mx = jnp.full((H, LANES), -jnp.inf, F32)
    for i in range(SK // KV_STEP):
        s = _nt(qa, ckv_v[pl.ds(i * KV_STEP, KV_STEP), :])
        s_v[:, pl.ds(i * KV_STEP, KV_STEP)] = s
        for j in range(KV_STEP // LANES):
            mx = jnp.maximum(mx, s[:, j * LANES:(j + 1) * LANES])
    mx = jnp.max(mx, axis=-1, keepdims=True)
    lsum = jnp.zeros((H, LANES), F32)
    lat = jnp.zeros((H, DC), F32)
    for i in range(SK // KV_STEP):
        p = jnp.exp(s_v[:, pl.ds(i * KV_STEP, KV_STEP)] - mx)
        for j in range(KV_STEP // LANES):
            lsum = lsum + p[:, j * LANES:(j + 1) * LANES]
        lat = lat + _nn(p.astype(BF16), ckv_v[pl.ds(i * KV_STEP, KV_STEP), :])
    lat = (lat / jnp.sum(lsum, axis=-1, keepdims=True)).astype(BF16)

    c_wuv.wait()
    ctx_v[...] = head_matvec(lat, wuv_v)
    ctx_flat = jnp.concatenate([ctx_v[pl.ds(h, 1), :] for h in range(H)], axis=1)
    ctx_flat = ctx_flat.astype(BF16)
    c_wo.wait()
    h1 = x + _nn(ctx_flat, wo_v[...])

    hn = _layernorm(h1).astype(BF16)
    c_w1.wait()
    c_b1.wait()
    pre = _nt(hn, w1_v[...]) + b1_v[...].astype(F32).reshape(1, FF)
    softplus = jnp.log1p(jnp.exp(-jnp.abs(pre))) + jnp.maximum(pre, 0.0)
    act = (pre * jnp.tanh(softplus)).astype(BF16)
    out = h1
    for c, (a, b) in zip(c_w2, w2_parts):
        c.wait()
        out = out + _nn(act[:, a:b], w2_v[pl.ds(a, b - a), :])
    o_ref[0] = out.astype(BF16)


def _kernel(*refs):
    pl.run_scoped(functools.partial(_body, *refs), pltpu.SemaphoreType.DMA((N_DMA,)))


@jax.jit
def pallas_sequential_preLN__compressed_kv_cla__dense_activation_mish__decode_kernel(
    A_x: jax.Array,
    A_c_kv: jax.Array,
    A_w_q: jax.Array,
    A_w_uk: jax.Array,
    A_w_uv: jax.Array,
    A_w_o: jax.Array,
    B_x: jax.Array,
    B_w1: jax.Array,
    B_b1: jax.Array,
    B_w2: jax.Array,
):
    del B_x
    hbm = pl.BlockSpec(memory_space=pltpu.HBM)
    return pl.pallas_call(
        _kernel,
        out_shape=jax.ShapeDtypeStruct((1, 1, M), BF16),
        in_specs=[hbm] * 9,
        out_specs=pl.BlockSpec(memory_space=pltpu.VMEM),
        scratch_shapes=[
            pltpu.VMEM((1, 1, M), BF16),
            pltpu.VMEM((FF,), BF16),
            pltpu.VMEM((SK, DC), BF16),
            pltpu.VMEM((M * H, D), BF16),
            pltpu.VMEM((DC * H, D), BF16),
            pltpu.VMEM((DC * H, D), BF16),
            pltpu.VMEM((H * D, M), BF16),
            pltpu.VMEM((FF, M), BF16),
            pltpu.VMEM((FF, M), BF16),
            pltpu.VMEM((H, SK), F32),
            pltpu.VMEM((H, D), F32),
        ],
        compiler_params=pltpu.CompilerParams(vmem_limit_bytes=64 * 1024 * 1024),
    )(
        A_x,
        A_c_kv.reshape(SK, DC),
        A_w_q.reshape(M * H, D),
        A_w_uk.reshape(DC * H, D),
        A_w_uv.reshape(DC * H, D),
        A_w_o.reshape(H * D, M),
        B_w1.T,
        B_b1,
        B_w2,
    )
```
